```python
import jax
import jax.numpy as jnp

def _softmax(x, axis=-1):
    return jax.nn.softmax(x, axis=axis)

def _gelu(x):
    return jax.nn.gelu(x, approximate=True)

def _silu(x):
    return jax.nn.silu(x)

def _sigmoid(x):
    return jax.nn.sigmoid(x)

def _layernorm(x, axis=-1, eps=1e-05):
    m = jnp.mean(x, axis=axis, keepdims=True)
    v = jnp.var(x, axis=axis, keepdims=True)
    return (x - m) / jnp.sqrt(v + eps)

def _scatter_add(tgt, idx, src, axis=0):
    return tgt.at[idx].add(src)

def _segment_sum(src, seg, n):
    return jax.ops.segment_sum(src, seg, n)

class _Rng:

    def __init__(self, key):
        self._k = key

    def _next(self):
        self._k, sub = jax.random.split(self._k)
        return sub

    def normal(self, shape):
        return jax.random.normal(self._next(), shape, dtype=jnp.bfloat16)

    def randint(self, lo, hi, shape):
        return jax.random.randint(self._next(), shape, lo, hi, dtype=jnp.int32)

    def uniform(self, shape, lo=0.0, hi=1.0):
        return jax.random.uniform(self._next(), shape, jnp.bfloat16, lo, hi)

    def permutation(self, n):
        return jax.random.permutation(self._next(), n)
kernel_name = 'adaLN_cond__grouped_kv_mqa__dense_activation_silu__prompt'

def _fwd_setup_inputs():
    _rng = _Rng(jax.random.key(int.from_bytes(__import__("os").urandom(4), "little")))
    _w = lambda a: (lambda t: t.astype(jnp.bfloat16) if jnp.issubdtype(t.dtype, jnp.floating) else t)(jnp.asarray(a))

    def _A_setup():
        B, S, D, H = (1, 2048, 640, 32)
        Dh = D // H
        return {'x': _w((lambda *s: _rng.normal(s) * 0.05)(B, S, D)), 'wq': _w((lambda *s: _rng.normal(s) * 0.05)(D, H * Dh)), 'wk': _w((lambda *s: _rng.normal(s) * 0.05)(D, Dh)), 'wv': _w((lambda *s: _rng.normal(s) * 0.05)(D, Dh)), 'wo': _w((lambda *s: _rng.normal(s) * 0.05)(H * Dh, D))}
    _A_in = _A_setup()

    def _B_setup():
        B, S, D, F = (1, 2048, 640, 1728)
        return {'x': _w((lambda *s: _rng.normal(s) * 0.05)(B, S, D)), 'w1': _w((lambda *s: _rng.normal(s) * 0.05)(D, F) * D ** (-0.5)), 'w2': _w((lambda *s: _rng.normal(s) * 0.05)(F, D) * F ** (-0.5))}
    _B_in = _B_setup()
    return {'A_x': _A_in['x'], 'A_wq': _A_in['wq'], 'A_wk': _A_in['wk'], 'A_wv': _A_in['wv'], 'A_wo': _A_in['wo'], 'B_x': _B_in['x'], 'B_w1': _B_in['w1'], 'B_w2': _B_in['w2'], 'c': _w((lambda *s: _rng.normal(s) * 0.05)(1, 640)), 'w_mod': _w((lambda *s: _rng.normal(s) * 0.05)(640, 6 * 640) * 640 ** (-0.5))}

def _fwd_reference(A_x, A_wq, A_wk, A_wv, A_wo, B_x, B_w1, B_w2, c, w_mod):

    def _A_ref(x, wq, wk, wv, wo):
        B, S, D = x.shape
        H = 32
        Dh = D // H
        q = (lambda x, *d: x.transpose(*d))((x @ wq).reshape(B, S, H, Dh), 0, 2, 1, 3)
        k = x @ wk
        v = x @ wv
        scores = jnp.einsum('bhqd,bkd->bhqk', q, k) * Dh ** (-0.5)
        p = _softmax(scores, axis=-1)
        o = jnp.einsum('bhqk,bkd->bhqd', p, v)
        return (lambda x, *d: x.transpose(*d))(o, 0, 2, 1, 3).reshape(B, S, H * Dh) @ wo

    def _B_ref(x, w1, w2):
        h = jnp.einsum('bsd,df->bsf', x, w1)
        h = _silu(h)
        out = jnp.einsum('bsf,fd->bsd', h, w2)
        return out
    x = A_x
    mod = (_silu(c) @ w_mod).reshape(c.shape[0], 6, 1, -1)
    sa, ca, ga, sb, cb, gb = (mod[:, 0].copy(), mod[:, 1].copy(), mod[:, 2].copy(), mod[:, 3].copy(), mod[:, 4].copy(), mod[:, 5].copy())
    h = _layernorm(x, axis=-1) * (1 + ca) + sa
    x = x + ga * _A_ref(h, A_wq, A_wk, A_wv, A_wo)
    h = _layernorm(x, axis=-1) * (1 + cb) + sb
    x = x + gb * _B_ref(h, B_w1, B_w2)
    return x

def setup_inputs():
    _inp = _fwd_setup_inputs()
    _gk = jax.random.fold_in(jax.random.key(int.from_bytes(__import__("os").urandom(4), "little")), 2 ** 31 - 1)
    _shapes = [[1, 2048, 640]]
    _dtypes = ['bfloat16']
    _gks = jax.random.split(_gk, len(_shapes))
    _gs = [jax.random.normal(k, s, dtype=jnp.dtype(d)) * 0.05 for k, s, d in zip(_gks, _shapes, _dtypes)]
    _inp['grad_out'] = _gs[0]
    return _inp

def reference(A_x, A_wq, A_wk, A_wv, A_wo, B_w1, B_w2, c, w_mod, B_x, grad_out):
    _const = dict(B_x=B_x)

    def _f(*_d):
        return _fwd_reference(**{'A_x': _d[0], 'A_wq': _d[1], 'A_wk': _d[2], 'A_wv': _d[3], 'A_wo': _d[4], 'B_w1': _d[5], 'B_w2': _d[6], 'c': _d[7], 'w_mod': _d[8], **_const})
    _out, _vjp = jax.vjp(_f, A_x, A_wq, A_wk, A_wv, A_wo, B_w1, B_w2, c, w_mod)
    _grads = _vjp(grad_out)
    _out0 = jnp.asarray(_out)
    return (_out0, *[jnp.asarray(_g) for _g in _grads])
```

```python
import math

import jax
import jax.numpy as jnp
import jax.experimental.pallas as pl
import jax.experimental.pallas.tpu as pltpu

f32 = jnp.float32
bf16 = jnp.bfloat16

S = 2048
D = 640
H = 32
DH = 20
DP = 32
F = 1728
TQ = 256
NB = S // TQ
GW = 512
HG = GW // TQ
G = H // HG
CK = 128
NC = S // CK
NJ = GW // 128
FP = 1792
FC = 256
NF = FP // FC
ND = D // 128
RC = 32
NRC = TQ // RC
FU = 2
BU = 4
NBL = G // BU
EPS = 1e-5
LOG2E = math.log2(math.e)
LN2 = math.log(2.0)
SCALE = DH ** (-0.5)

NT = (((1,), (1,)), ((), ()))
TN = (((0,), (0,)), ((), ()))


def _dot(a, b):
    return jnp.dot(a, b, preferred_element_type=f32)


def _dot_nt(a, b):
    return jax.lax.dot_general(a, b, NT, preferred_element_type=f32)


def _dot_tn(a, b):
    return jax.lax.dot_general(a, b, TN, preferred_element_type=f32)


def _sigmoid(x):
    return 1.0 / (1.0 + jnp.exp(-x))


def _ln_stats(x):
    m = jnp.mean(x, axis=-1, keepdims=True)
    xc = x - m
    v = jnp.mean(xc * xc, axis=-1, keepdims=True)
    rstd = jax.lax.rsqrt(v + EPS)
    return xc * rstd, rstd


def _ln_bwd(dy, xhat, rstd):
    m1 = jnp.mean(dy, axis=-1, keepdims=True)
    m2 = jnp.mean(dy * xhat, axis=-1, keepdims=True)
    return rstd * (dy - m1 - xhat * m2)


def _colsum(x):
    return jnp.sum(x, axis=0, keepdims=True)


def _colsum8(x):
    return jnp.sum(x.reshape(x.shape[0] // 8, 8, x.shape[1]), axis=0)


def _kernel(x_hbm, wq_hbm, wkT_ref, wvT_ref, wo_hbm, w1T_hbm, w2_hbm, c_ref,
            wmod_hbm, g_hbm,
            out_hbm, dx_hbm, dwq_hbm, dwkT_ref, dwvT_ref, dwo_hbm, dw1T_hbm,
            dw2_hbm, dc_ref, dwmod_hbm,
            x_ref, wq_ref, wo_ref, w1T_ref, w2_ref, wmod_ref, g_ref,
            out_ref, dx_ref, dwq_ref, dwo_ref, dw1T_ref, dw2_ref, dwmod_ref,
            sem_in, sem_x, sem_out, sem_dx, sem_w,
            mod_s, h1_s, wqT_s, wkvT_s, kaug_s, vaug_s, kT_s, vT_s,
            p_s, s_s, m_s, qt_s, pad_s, t640_s, ot_s, invl_s,
            dot_s, dqt_s, dkT_s, dvT_s, dw1_s, dw2_s, dwo_s, dwqT_s, dmod_s,
            dx1_s, dh1_s, dp_s, h2_s, df_s, x1_s, at_s, f_s, dh2_s,
            a_s, du_s, t640b_s, xh_s, rstd_s, dat_s, scol_s, xh1_s, rstd1_s):
    def blk(b):
        return pl.ds(pl.multiple_of(b * TQ, TQ), TQ)

    def rchunk(b, rc):
        return pl.ds(pl.multiple_of(b * TQ + rc * RC, RC), RC)

    def x_copy(b):
        return pltpu.make_async_copy(x_hbm.at[blk(b), :], x_ref.at[blk(b), :], sem_x.at[b])

    def out_copy(b):
        return pltpu.make_async_copy(out_ref.at[blk(b), :], out_hbm.at[blk(b), :], sem_out.at[b])

    def dx_copy(b):
        return pltpu.make_async_copy(dx_ref.at[blk(b), :], dx_hbm.at[blk(b), :], sem_dx.at[b])

    cp_wmod0 = pltpu.make_async_copy(wmod_hbm.at[:, 0:2 * D], wmod_ref.at[:, 0:2 * D], sem_in.at[0])
    cp_wq = pltpu.make_async_copy(wq_hbm, wq_ref, sem_in.at[1])
    cp_wmod1 = pltpu.make_async_copy(wmod_hbm.at[:, 2 * D:6 * D], wmod_ref.at[:, 2 * D:6 * D], sem_in.at[2])
    cp_wo = pltpu.make_async_copy(wo_hbm, wo_ref, sem_in.at[3])
    cp_w1 = pltpu.make_async_copy(w1T_hbm, w1T_ref.at[0:F, :], sem_in.at[4])
    cp_w2 = pltpu.make_async_copy(w2_hbm, w2_ref.at[0:F, :], sem_in.at[5])
    cp_g = pltpu.make_async_copy(g_hbm, g_ref, sem_in.at[6])
    cp_dwq = pltpu.make_async_copy(dwq_ref, dwq_hbm, sem_w.at[0])
    cp_dwo = pltpu.make_async_copy(dwo_ref, dwo_hbm, sem_w.at[1])
    cp_dw1 = pltpu.make_async_copy(dw1T_ref, dw1T_hbm, sem_w.at[2])
    cp_dw2 = pltpu.make_async_copy(dw2_ref, dw2_hbm, sem_w.at[3])
    cp_dwmod0 = pltpu.make_async_copy(dwmod_ref.at[:, 0:2 * D], dwmod_hbm.at[:, 0:2 * D], sem_w.at[4])
    cp_dwmod1 = pltpu.make_async_copy(dwmod_ref.at[:, 2 * D:6 * D], dwmod_hbm.at[:, 2 * D:6 * D], sem_w.at[5])

    cp_wmod0.start()
    cp_wq.start()
    x_copy(0).start()

    dkT_s[...] = jnp.zeros_like(dkT_s)
    dvT_s[...] = jnp.zeros_like(dvT_s)
    dw1_s[...] = jnp.zeros_like(dw1_s)
    dw2_s[...] = jnp.zeros_like(dw2_s)
    dwo_s[...] = jnp.zeros_like(dwo_s)
    dwqT_s[...] = jnp.zeros_like(dwqT_s)
    dmod_s[...] = jnp.zeros_like(dmod_s)
    pad_s[...] = jnp.zeros_like(pad_s)
    dqt_s[...] = jnp.zeros_like(dqt_s)
    f_s[...] = jnp.zeros_like(f_s)
    dh2_s[...] = jnp.zeros_like(dh2_s)
    w1T_ref[F:FP, :] = jnp.zeros((FP - F, D), bf16)
    w2_ref[F:FP, :] = jnp.zeros((FP - F, D), bf16)

    c = c_ref[...].astype(f32)
    sig_c = _sigmoid(c)
    silu_c = c * sig_c
    silu_b = silu_c.astype(bf16)
    scol_s[...] = jnp.broadcast_to(silu_c, (128, D)).T
    cp_wmod0.wait()
    for b in range(1, NB):
        x_copy(b).start()
    mod_s[:, 0:2 * D] = _dot(silu_b, wmod_ref[:, 0:2 * D])

    def mod(i):
        return mod_s[:, i * D:(i + 1) * D]

    zrow = jnp.zeros((DP - DH, D), f32)
    wkvT_s[...] = jnp.concatenate(
        [wkT_ref[...].astype(f32), zrow, wvT_ref[...].astype(f32), zrow],
        axis=0).astype(bf16)

    col_id = jax.lax.broadcasted_iota(jnp.int32, (128, DP), 1)
    ones_cols = jnp.where((col_id >= DH) & (col_id < DH + 3), 1.0, 0.0)
    row_id = jax.lax.broadcasted_iota(jnp.int32, (DP, 128), 0)
    ones_row = jnp.where(row_id == DH, 1.0, 0.0)

    def expand(src_ref, dst_ref):
        for hh in range(H):
            g, j = hh // HG, hh % HG
            dst_ref[g, 0:DH, j * TQ:(j + 1) * TQ] = src_ref[DH * hh:DH * (hh + 1), :]

    def compact(src_ref, dst_ref):
        for hh in range(H):
            g, j = hh // HG, hh % HG
            dst_ref[DH * hh:DH * (hh + 1), :] = src_ref[g, 0:DH, j * TQ:(j + 1) * TQ]

    cp_wq.wait()
    wqT_s[...] = wq_ref[...].T

    def phase_a(b, carry):
        r0 = pl.multiple_of(b * TQ, TQ)
        rows = pl.ds(r0, TQ)
        x_copy(b).wait()
        for hf in range(TQ // 128):
            hr = pl.ds(pl.multiple_of(b * TQ + hf * 128, 128), 128)
            hs = slice(hf * 128, (hf + 1) * 128)
            xhat, rstd = _ln_stats(x_ref[hr, :].astype(f32))
            xh1_s[hr, :] = xhat
            rstd1_s[hr, :] = rstd
            h1 = (xhat * (1.0 + mod(1)) + mod(0)).astype(bf16)
            h1_s[hr, :] = h1
            kvT = _dot_nt(wkvT_s[...], h1)
            kT_s[:, hr] = kvT[0:DP].astype(bf16)
            vT_s[:, hr] = (kvT[DP:2 * DP] + ones_row).astype(bf16)
            kaug_s[hr, :] = kvT[0:DP].T.astype(bf16)
            vaug_s[hr, :] = (kvT[DP:2 * DP].T + ones_cols).astype(bf16)
            t640_s[:, hs] = _dot_nt(wqT_s[...], h1) * (SCALE * LOG2E)
        expand(t640_s, pad_s)
        qt_s[pl.ds(pl.multiple_of(b * G, G), G)] = pad_s[...].astype(bf16)
        return carry

    with jax.named_scope('phase_a'):
        jax.lax.fori_loop(0, NB, phase_a, 0)

    cp_wmod1.start()
    cp_wo.start()
    cp_w1.start()
    cp_w2.start()
    cp_g.start()

    grow_id = jax.lax.broadcasted_iota(jnp.int32, (DP, GW), 0)
    row8 = jax.lax.broadcasted_iota(jnp.int32, (8, GW), 0)
    hrow = jax.lax.broadcasted_iota(jnp.int32, (H, D), 0)
    hcol = jax.lax.broadcasted_iota(jnp.int32, (H, D), 1)
    head_ind = jnp.where((hcol >= hrow * DH) & (hcol < (hrow + 1) * DH),
                         1.0, 0.0).astype(bf16)

    def finish_o(gc, o):
        inv_l = 1.0 / o[DH:DH + 1, :]
        invl_s[gc] = inv_l
        ot_s[gc] = jnp.where(grow_id < DH, o * inv_l, 0.0)

    def fwd_step(b, tc, consume):
        qbase = jnp.minimum(b * G + (tc + 1) * FU, NB * G - FU)
        for u in range(FU):
            qn = qt_s[qbase + u]
            if consume:
                gc = tc * FU + u
                mc = m_s[u]
            m8 = None
            o = None
            for ck in range(NC):
                sl = slice(ck * CK, (ck + 1) * CK)
                if consume:
                    p = jnp.exp2(s_s[u, sl, :] - mc).astype(bf16)
                    p_s[gc, sl, :] = p
                s = _dot(kaug_s[sl, :], qn)
                s_s[u, sl, :] = s
                mm = jnp.max(s.reshape(CK // 8, 8, GW), axis=0)
                m8 = mm if m8 is None else jnp.maximum(m8, mm)
                if consume:
                    oo = _dot(vT_s[:, sl], p)
                    o = oo if o is None else o + oo
            m_s[u] = jnp.max(m8, axis=0, keepdims=True)
            if consume:
                finish_o(gc, o)

    def bwd_group(b, gg):
        dp = dp_s[...]
        for u in range(BU):
            g = gg * BU + u
            q = qt_s[b * G + g]
            do = dot_s[g]
            dq = None
            for ck in range(NC):
                sl = slice(ck * CK, (ck + 1) * CK)
                p = p_s[g, sl, :]
                ds = (p.astype(f32) * dp).astype(bf16)
                if ck + 1 < NC:
                    dp = _dot(vaug_s[(ck + 1) * CK:(ck + 2) * CK, :], do)
                else:
                    gnext = jnp.minimum(g + 1, G - 1)
                    dp = _dot(vaug_s[0:CK, :], dot_s[gnext])
                dv = None
                for j in range(NJ):
                    js = slice(j * 128, (j + 1) * 128)
                    t = _dot_nt(do[:, js], p[:, js])
                    dv = t if dv is None else dv + t
                dk = None
                for j in range(NJ):
                    js = slice(j * 128, (j + 1) * 128)
                    t = _dot_nt(q[:, js], ds[:, js])
                    dk = t if dk is None else dk + t
                dvT_s[:, sl] += dv
                dkT_s[:, sl] += dk
                d = _dot(kT_s[:, sl], ds)
                dq = d if dq is None else dq + d
            dqt_s[g] = dq
        dp_s[...] = dp

    def fchunk(j):
        if isinstance(j, int):
            return slice(j * FC, (j + 1) * FC)
        return pl.ds(pl.multiple_of(j * FC, FC), FC)

    def ffn_act(u, da):
        sig = _sigmoid(u)
        a = (u * sig).astype(bf16)
        du = (da * (sig * (1.0 + u * (1.0 - sig)))).astype(bf16)
        return a, du

    def dq_compact():
        compact(dqt_s, t640b_s)
        return (t640b_s[...] * SCALE).astype(bf16)

    def phase_b(b, carry):
        rows = blk(b)
        prev = blk(jnp.maximum(b - 1, 0))

        def fwd_body(t, cc):
            fwd_step(b, t, True)
            return cc

        with jax.named_scope('fwd_loop'):
            jax.lax.fori_loop(0, G // FU, fwd_body, 0)

        @pl.when(b == 0)
        def _():
            cp_wmod1.wait()
            mod_s[:, 2 * D:6 * D] = _dot(silu_b, wmod_ref[:, 2 * D:6 * D])
            cp_wo.wait()
            cp_w1.wait()
            cp_w2.wait()
            cp_g.wait()

        compact(ot_s, t640_s)
        ob = t640_s[...].T.astype(bf16)
        dqT = dq_compact()
        dq = dqT.T

        ga, sb, cb, gb = mod(2), mod(3), mod(4), mod(5)
        df = (g_ref[rows, :].astype(f32) * gb).astype(bf16)
        df_s[...] = df
        da = _dot_nt(df, w2_ref[fchunk(0), :])

        def act0(rc0):
            r2 = slice(rc0 * RC, (rc0 + 2) * RC)
            u = _dot_nt(h2_s[r2, :], w1T_ref[fchunk(0), :])
            a, du = ffn_act(u, da[r2, :])
            a_s[r2, :] = a
            du_s[r2, :] = du

        for rc in range(NRC):
            rs = slice(rc * RC, (rc + 1) * RC)
            attn = _dot(ob[rs, :], wo_ref[...])
            at_s[rs, :] = attn
            x1 = x_ref[rchunk(b, rc), :].astype(f32) + ga * attn
            xhat2, rstd2 = _ln_stats(x1)
            h2_s[rs, :] = (xhat2 * (1.0 + cb) + sb).astype(bf16)
            x1_s[rs, :] = x1
            xh_s[rs, :] = xhat2
            rstd_s[rs, :] = rstd2
            if rc < ND:
                ns = slice(rc * 128, (rc + 1) * 128)
                dh1_s[prev, ns] = _dot(dq, wqT_s[:, ns])
            else:
                ms = slice((rc - ND) * 128, (rc - ND + 1) * 128)
                dwqT_s[ms, :] += _dot(dqT[ms, :], h1_s[prev, :])
            if rc % 2 == 1 and rc >= 3:
                act0(rc - 3)
        ms = slice((NRC - ND) * 128, (NRC - ND + 1) * 128)
        dwqT_s[ms, :] += _dot(dqT[ms, :], h1_s[prev, :])
        act0(NRC - 2)
        ms = slice((NRC - ND + 1) * 128, D)
        dwqT_s[ms, :] += _dot(dqT[ms, :], h1_s[prev, :])

        def ffn(j, cc):
            fs = fchunk(j)
            fn = fchunk(j + 1)
            h2v = h2_s[...]
            dfv = df_s[...]
            a = a_s[...]
            du = du_s[...]
            f_s[...] = jnp.where(j > 0, f_s[...], 0.0) + _dot(a, w2_ref[fs, :])
            dh2_s[...] = jnp.where(j > 0, dh2_s[...], 0.0) + _dot(du, w1T_ref[fs, :])
            un = _dot_nt(h2v, w1T_ref[fn, :])
            dan = _dot_nt(dfv, w2_ref[fn, :])
            an, dun = ffn_act(un, dan)
            a_s[...] = an
            du_s[...] = dun
            dw2_s[fs, :] += _dot_tn(a, dfv)
            dw1_s[fs, :] += _dot_tn(du, h2v)
            return cc

        with jax.named_scope('ffn'):
            jax.lax.fori_loop(0, NF - 1, ffn, 0)

        fs = fchunk(NF - 1)
        a = a_s[...]
        du = du_s[...]
        aT = a.T
        duT = du.T

        for rc in range(NRC):
            rs = slice(rc * RC, (rc + 1) * RC)
            rr = rchunk(b, rc)
            dh2 = dh2_s[rs, :] + _dot(du[rs, :], w1T_ref[fs, :])
            f = f_s[rs, :] + _dot(a[rs, :], w2_ref[fs, :])
            xhat2 = xh_s[rs, :]
            gr = g_ref[rr, :].astype(f32)
            out_ref[rr, :] = (x1_s[rs, :] + gb * f).astype(out_ref.dtype)
            dmod_s[:, 5 * D:6 * D] += _colsum8(gr * f)
            dmod_s[:, 3 * D:4 * D] += _colsum8(dh2)
            dmod_s[:, 4 * D:5 * D] += _colsum8(dh2 * xhat2)
            dx1 = gr + _ln_bwd(dh2 * (1.0 + cb), xhat2, rstd_s[rs, :])
            dx1_s[rr, :] = dx1
            dmod_s[:, 2 * D:3 * D] += _colsum8(dx1 * at_s[rs, :])
            dat_s[rs, :] = (dx1 * ga).astype(bf16)
            if rc < ND:
                ns = slice(rc * 128, (rc + 1) * 128)
                dw2_s[fs, ns] += _dot(aT, df_s[:, ns])
                dw1_s[fs, ns] += _dot(duT, h2_s[:, ns])
        out_copy(b).start()
        dattn = dat_s[...]
        t640b_s[...] = _dot_nt(wo_ref[...], dattn)
        dwo_s[0:256, :] += _dot(t640_s[0:256, :].astype(bf16), dattn)
        expand(t640b_s, pad_s)
        prod = t640b_s[...] * t640_s[...]
        prod_hi = prod.astype(bf16)
        prod_lo = (prod - prod_hi.astype(f32)).astype(bf16)
        delta = _dot(head_ind, prod_hi) + _dot(head_ind, prod_lo)
        for hh in range(H):
            g, j = hh // HG, hh % HG
            pad_s[g, DH:DH + 1, j * TQ:(j + 1) * TQ] = -delta[hh:hh + 1, :]

        for g in range(G):
            v = pad_s[g] * invl_s[g]
            top = v[16:24, :]
            r1 = top - top.astype(bf16).astype(f32)
            r2 = r1 - r1.astype(bf16).astype(f32)
            top = jnp.where(row8 == DH + 1 - 16, pltpu.roll(r1, 1, 0),
                            jnp.where(row8 == DH + 2 - 16, pltpu.roll(r2, 2, 0), top))
            dot_s[g] = jnp.concatenate([v[0:16], top, v[24:32]], axis=0).astype(bf16)

        dwo_s[256:D, :] += _dot(t640_s[256:D, :].astype(bf16), dattn)
        dp_s[...] = _dot(vaug_s[0:CK, :], dot_s[0])

        @pl.when(b == NB - 1)
        def _():
            dwo_ref[...] = dwo_s[...].astype(bf16)
            cp_dwo.start()
            dw1T_ref[...] = dw1_s[0:F, :].astype(bf16)
            cp_dw1.start()
            dw2_ref[...] = dw2_s[0:F, :].astype(bf16)
            cp_dw2.start()
            dmr = _colsum(dmod_s[:, 2 * D:6 * D])
            sc = scol_s[...]
            for n in range(4 * ND):
                ns = slice((2 * ND + n) * 128, (2 * ND + n + 1) * 128)
                dwmod_ref[:, ns] = (sc * dmr[:, n * 128:(n + 1) * 128]).astype(bf16)
            cp_dwmod1.start()

        def bwd_body(gg, cc):
            bwd_group(b, gg)
            return cc

        with jax.named_scope('bwd_loop'):
            jax.lax.fori_loop(0, NBL, bwd_body, 0)
        return carry

    fwd_step(0, -1, False)
    with jax.named_scope('phase_b'):
        jax.lax.fori_loop(0, NB, phase_b, 0)

    last = slice((NB - 1) * TQ, NB * TQ)
    dqT = dq_compact()
    dh1_s[last, :] = _dot_tn(dqT, wqT_s[...])
    dwqT_s[...] += _dot(dqT, h1_s[last, :])

    dwq_ref[...] = dwqT_s[...].T.astype(dwq_ref.dtype)
    cp_dwq.start()
    srow_id = jax.lax.broadcasted_iota(jnp.int32, (DP, S), 0)
    dkT = jnp.where(srow_id < DH, dkT_s[...] * LN2, 0.0).astype(bf16)
    dvT = jnp.where(srow_id < DH, dvT_s[...], 0.0).astype(bf16)
    kaug_s[...] = dkT.T
    vaug_s[...] = dvT.T
    dwkT = _dot(dkT, h1_s[...])
    dwvT = _dot(dvT, h1_s[...])
    dwkT_ref[...] = dwkT[0:DH, :].astype(dwkT_ref.dtype)
    dwvT_ref[...] = dwvT[0:DH, :].astype(dwvT_ref.dtype)

    def phase_c(b, carry):
        ca1 = 1.0 + mod(1)
        for hf in range(TQ // 64):
            hr = pl.ds(pl.multiple_of(b * TQ + hf * 64, 64), 64)
            dh1 = dh1_s[hr, :] + _dot(kaug_s[hr, :], wkvT_s[0:DP, :]) \
                + _dot(vaug_s[hr, :], wkvT_s[DP:2 * DP, :])
            xhat = xh1_s[hr, :]
            dmod_s[:, 0:D] += _colsum8(dh1)
            dmod_s[:, D:2 * D] += _colsum8(dh1 * xhat)
            dx = dx1_s[hr, :] + _ln_bwd(dh1 * ca1, xhat, rstd1_s[hr, :])
            dx_ref[hr, :] = dx.astype(dx_ref.dtype)
        dx_copy(b).start()
        return carry

    with jax.named_scope('phase_c'):
        jax.lax.fori_loop(0, NB, phase_c, 0)

    dmod32 = _colsum(dmod_s[...])
    dmod = dmod32.astype(bf16)
    sc = scol_s[...]
    for n in range(2 * ND):
        ns = slice(n * 128, (n + 1) * 128)
        dwmod_ref[:, ns] = (sc * dmod32[:, ns]).astype(bf16)
    cp_dwmod0.start()
    dsilu = _dot_nt(dmod, wmod_ref[...])
    dc_ref[...] = (dsilu * (sig_c * (1.0 + c * (1.0 - sig_c)))).astype(dc_ref.dtype)

    for b in range(NB):
        out_copy(b).wait()
        dx_copy(b).wait()
    cp_dwq.wait()
    cp_dwo.wait()
    cp_dw1.wait()
    cp_dw2.wait()
    cp_dwmod0.wait()
    cp_dwmod1.wait()


@jax.jit
def pallas_adaLN_cond__grouped_kv_mqa__dense_activation_silu__prompt_kernel(
    A_x: jax.Array,
    A_wq: jax.Array,
    A_wk: jax.Array,
    A_wv: jax.Array,
    A_wo: jax.Array,
    B_x: jax.Array,
    B_w1: jax.Array,
    B_w2: jax.Array,
    c: jax.Array,
    w_mod: jax.Array,
    grad_out: jax.Array,
):
    x = A_x.reshape(S, D)
    g = grad_out.reshape(S, D)
    sds = jax.ShapeDtypeStruct
    out_shape = (
        sds((S, D), bf16),
        sds((S, D), bf16),
        sds((D, D), bf16),
        sds((DH, D), bf16),
        sds((DH, D), bf16),
        sds((D, D), bf16),
        sds((F, D), bf16),
        sds((F, D), bf16),
        sds((1, D), bf16),
        sds((D, 6 * D), bf16),
    )
    V = pltpu.VMEM
    DMA = pltpu.SemaphoreType.DMA
    scratch = [
        V((S, D), bf16),
        V((D, D), bf16),
        V((D, D), bf16),
        V((FP, D), bf16),
        V((FP, D), bf16),
        V((D, 6 * D), bf16),
        V((S, D), bf16),
        V((S, D), bf16),
        V((S, D), bf16),
        V((D, D), bf16),
        V((D, D), bf16),
        V((F, D), bf16),
        V((F, D), bf16),
        V((D, 6 * D), bf16),
        DMA((7,)),
        DMA((NB,)),
        DMA((NB,)),
        DMA((NB,)),
        DMA((6,)),
        V((1, 6 * D), f32),
        V((S, D), bf16),
        V((D, D), bf16),
        V((2 * DP, D), bf16),
        V((S, DP), bf16),
        V((S, DP), bf16),
        V((DP, S), bf16),
        V((DP, S), bf16),
        V((G, S, GW), bf16),
        V((FU, S, GW), f32),
        V((FU, 1, GW), f32),
        V((NB * G, DP, GW), bf16),
        V((G, DP, GW), f32),
        V((D, TQ), f32),
        V((G, DP, GW), f32),
        V((G, 1, GW), f32),
        V((G, DP, GW), bf16),
        V((G, DP, GW), f32),
        V((DP, S), f32),
        V((DP, S), f32),
        V((FP, D), f32),
        V((FP, D), f32),
        V((D, D), f32),
        V((D, D), f32),
        V((8, 6 * D), f32),
        V((S, D), f32),
        V((S, D), f32),
        V((CK, GW), f32),
        V((TQ, D), bf16),
        V((TQ, D), bf16),
        V((TQ, D), f32),
        V((TQ, D), f32),
        V((TQ, D), f32),
        V((TQ, D), f32),
        V((TQ, FC), bf16),
        V((TQ, FC), bf16),
        V((D, TQ), f32),
        V((TQ, D), f32),
        V((TQ, 1), f32),
        V((TQ, D), bf16),
        V((D, 128), f32),
        V((S, D), f32),
        V((S, 1), f32),
    ]
    hbm = pl.BlockSpec(memory_space=pl.ANY)
    vm = pl.BlockSpec(memory_space=pltpu.VMEM)
    outs = pl.pallas_call(
        _kernel,
        out_shape=out_shape,
        in_specs=[hbm, hbm, vm, vm, hbm, hbm, hbm, vm, hbm, hbm],
        out_specs=(hbm, hbm, hbm, vm, vm, hbm, hbm, hbm, vm, hbm),
        scratch_shapes=scratch,
        compiler_params=pltpu.CompilerParams(
            vmem_limit_bytes=126 * 1024 * 1024),
    )(x, A_wq, A_wk.T, A_wv.T, A_wo, B_w1.T, B_w2, c, w_mod, g)
    out, dx = outs[0].reshape(1, S, D), outs[1].reshape(1, S, D)
    return (out, dx, outs[2], outs[3].T, outs[4].T, outs[5], outs[6].T,
            outs[7], outs[8], outs[9])
```

```python
import math

import jax
import jax.numpy as jnp
import jax.experimental.pallas as pl
import jax.experimental.pallas.tpu as pltpu

f32 = jnp.float32
bf16 = jnp.bfloat16

S = 2048
D = 640
H = 32
DH = 20
DP = 32
DQ = 24
F = 1728
TQ = 256
NB = S // TQ
GW = 512
HG = GW // TQ
G = H // HG
CK = 128
NC = S // CK
NJ = GW // 128
FP = 1792
FC = 256
NF = FP // FC
FUN = 3
ND = D // 128
RC = 32
NRC = TQ // RC
FU = 4
BU = 4
NBL = G // BU
EPS = 1e-5
LOG2E = math.log2(math.e)
LN2 = math.log(2.0)
SCALE = DH ** (-0.5)

NN = (((1,), (0,)), ((), ()))
NT = (((1,), (1,)), ((), ()))
TN = (((0,), (0,)), ((), ()))


def _dot(a, b):
    return jnp.dot(a, b, preferred_element_type=f32)


def _dot_nn(a, b):
    return jax.lax.dot_general(a, b, NN, preferred_element_type=f32)


def _r32(x):
    return x.astype(bf16).astype(f32)


def _dot_nt(a, b):
    return jax.lax.dot_general(a, b, NT, preferred_element_type=f32)


def _dot_tn(a, b):
    return jax.lax.dot_general(a, b, TN, preferred_element_type=f32)


def _sigmoid(x):
    return 1.0 / (1.0 + jnp.exp(-x))


def _ln_stats(x):
    m = jnp.mean(x, axis=-1, keepdims=True)
    xc = x - m
    v = jnp.mean(xc * xc, axis=-1, keepdims=True)
    rstd = jax.lax.rsqrt(v + EPS)
    return xc * rstd, rstd


def _ln_bwd(dy, xhat, rstd):
    m1 = jnp.mean(dy, axis=-1, keepdims=True)
    m2 = jnp.mean(dy * xhat, axis=-1, keepdims=True)
    return rstd * (dy - m1 - xhat * m2)


def _colsum(x):
    return jnp.sum(x, axis=0, keepdims=True)


def _colsum8(x):
    return jnp.sum(x.reshape(x.shape[0] // 8, 8, x.shape[1]), axis=0)


def _kernel(x_hbm, wq_hbm, wkT_ref, wvT_ref, wo_hbm, w1T_hbm, w2_hbm, c_ref,
            wmod_hbm, g_hbm,
            out_hbm, dx_hbm, dwq_hbm, dwkT_ref, dwvT_ref, dwo_hbm, dw1T_hbm,
            dw2_hbm, dc_ref, dwmod_hbm,
            x_ref, wo_ref, w1T_ref, w2_ref, wmod_ref, g_ref,
            out_ref, dwq_ref, dwo_ref, dw1T_ref, dw2_ref, dwmod_ref,
            sem_in, sem_g, sem_x, sem_out, sem_dx, sem_w,
            mod_s, h1_s, wqT_s, wkvT_s, kaug_s, vaug_s, kT_s, vT_s,
            p_s, s_s, m_s, qt_s, pad_s, t640_s, ot_s, invl_s,
            dot_s, dqt_s, dkT_s, dvT_s, dw1_s, dw2_s, dwo_s, dwqT_s, dmod_s,
            dx1_s, dh1_s, dp_s, h2_s, df_s, x1_s, at_s, f_s, dh2_s,
            a_s, du_s, t640b_s, xh_s, rstd_s, dat_s, scol_s, xh1_s, rstd1_s, dsl_s):
    wq_ref = dwq_ref
    dx_ref = out_ref

    def blk(b):
        return pl.ds(pl.multiple_of(b * TQ, TQ), TQ)

    def rchunk(b, rc):
        return pl.ds(pl.multiple_of(b * TQ + rc * RC, RC), RC)

    def x_copy(b):
        return pltpu.make_async_copy(x_hbm.at[blk(b), :], x_ref.at[blk(b), :], sem_x.at[b])

    def g_copy(b):
        return pltpu.make_async_copy(g_hbm.at[blk(b), :], g_ref.at[b % 2], sem_g.at[b % 2])

    def out_copy(b):
        return pltpu.make_async_copy(out_ref.at[blk(b), :], out_hbm.at[blk(b), :], sem_out.at[b])

    def dx_copy(b):
        return pltpu.make_async_copy(dx_ref.at[blk(b), :], dx_hbm.at[blk(b), :], sem_dx.at[b])

    cp_wmod0 = pltpu.make_async_copy(wmod_hbm.at[:, 0:2 * D], wmod_ref.at[:, 0:2 * D], sem_in.at[0])
    cp_wq = pltpu.make_async_copy(wq_hbm, wq_ref, sem_in.at[1])
    cp_wmod1 = pltpu.make_async_copy(wmod_hbm.at[:, 2 * D:6 * D], wmod_ref.at[:, 2 * D:6 * D], sem_in.at[2])
    cp_wo = pltpu.make_async_copy(wo_hbm, wo_ref, sem_in.at[3])
    cp_w1 = pltpu.make_async_copy(w1T_hbm, w1T_ref.at[0:F, :], sem_in.at[4])
    cp_w2 = pltpu.make_async_copy(w2_hbm, w2_ref.at[0:F, :], sem_in.at[5])
    cp_dwq = pltpu.make_async_copy(dwq_ref, dwq_hbm, sem_w.at[0])
    cp_dwo = pltpu.make_async_copy(dwo_ref, dwo_hbm, sem_w.at[1])
    cp_dw1 = pltpu.make_async_copy(dw1T_ref, dw1T_hbm, sem_w.at[2])
    cp_dw2 = pltpu.make_async_copy(dw2_ref, dw2_hbm, sem_w.at[3])
    cp_dwmod0 = pltpu.make_async_copy(dwmod_ref, dwmod_hbm.at[:, 0:2 * D], sem_w.at[4])
    cp_dwmod1 = pltpu.make_async_copy(wmod_ref.at[:, 2 * D:6 * D], dwmod_hbm.at[:, 2 * D:6 * D], sem_w.at[5])

    cp_wmod0.start()
    cp_wq.start()
    x_copy(0).start()

    dkT_s[...] = jnp.zeros_like(dkT_s)
    dvT_s[...] = jnp.zeros_like(dvT_s)

    def zero_acc(i, cc):
        fr = pl.ds(pl.multiple_of(i * (FP // 8), 8), FP // 8)
        dw1_s[fr, :] = jnp.zeros((FP // 8, D), f32)
        dw2_s[fr, :] = jnp.zeros((FP // 8, D), f32)
        dr = pl.ds(pl.multiple_of(i * (D // 8), 8), D // 8)
        dwo_s[dr, :] = jnp.zeros((D // 8, D), f32)
        dwqT_s[dr, :] = jnp.zeros((D // 8, D), f32)
        tr = pl.ds(pl.multiple_of(i * (TQ // 8), 8), TQ // 8)
        f_s[tr, :] = jnp.zeros((TQ // 8, D), f32)
        dh2_s[tr, :] = jnp.zeros((TQ // 8, D), f32)
        gr = pl.ds(i * (G // 8), G // 8)
        pad_s[gr] = jnp.zeros((G // 8, DP, GW), f32)
        dqt_s[gr] = jnp.zeros((G // 8, DQ, GW), f32)
        return cc

    jax.lax.fori_loop(0, 8, zero_acc, 0)
    dmod_s[...] = jnp.zeros_like(dmod_s)
    w1T_ref[F:FP, :] = jnp.zeros((FP - F, D), bf16)
    w2_ref[F:FP, :] = jnp.zeros((FP - F, D), bf16)

    c = c_ref[...].astype(f32)
    sig_c = _sigmoid(c)
    silu_c = c * sig_c
    silu_b = silu_c.astype(bf16)
    scol_s[...] = jnp.broadcast_to(silu_c, (128, D)).T
    cp_wmod0.wait()
    for b in range(1, NB):
        x_copy(b).start()
    mod_s[:, 0:2 * D] = _dot(silu_b, wmod_ref[:, 0:2 * D])

    def mod(i):
        return mod_s[:, i * D:(i + 1) * D]

    zrow = jnp.zeros((DP - DH, D), f32)
    wkvT_s[...] = jnp.concatenate(
        [wkT_ref[...].astype(f32), zrow, wvT_ref[...].astype(f32), zrow],
        axis=0).astype(bf16)

    col_id = jax.lax.broadcasted_iota(jnp.int32, (128, DP), 1)
    ones_cols = jnp.where((col_id >= DH) & (col_id < DH + 3), 1.0, 0.0)
    row_id = jax.lax.broadcasted_iota(jnp.int32, (DQ, 128), 0)
    ones_row = jnp.where(row_id == DH, 1.0, 0.0)

    def expand(src_ref, dst_ref):
        for hh in range(H):
            g, j = hh // HG, hh % HG
            dst_ref[g, 0:DH, j * TQ:(j + 1) * TQ] = src_ref[DH * hh:DH * (hh + 1), :]

    def compact(src_ref, dst_ref):
        for hh in range(H):
            g, j = hh // HG, hh % HG
            dst_ref[DH * hh:DH * (hh + 1), :] = src_ref[g, 0:DH, j * TQ:(j + 1) * TQ]

    cp_wq.wait()
    wqT_s[...] = wq_ref[...].T

    def phase_a(b, carry):
        x_copy(b).wait()
        for hf in range(TQ // 128):
            hr = pl.ds(pl.multiple_of(b * TQ + hf * 128, 128), 128)
            hs = slice(hf * 128, (hf + 1) * 128)
            xhat, rstd = _ln_stats(x_ref[hr, :].astype(f32))
            xh1_s[hr, :] = xhat
            rstd1_s[hr, :] = rstd
            h1 = (xhat * (1.0 + mod(1)) + mod(0)).astype(bf16)
            h1_s[hr, :] = h1
            kvT = _dot_nt(wkvT_s[...], h1)
            kT_s[:, hr] = _r32(kvT[0:DQ])
            vT_s[:, hr] = _r32(kvT[DP:DP + DQ] + ones_row)
            kaug_s[hr, :] = kvT[0:DP].T.astype(bf16)
            vaug_s[hr, :] = (kvT[DP:2 * DP].T + ones_cols).astype(bf16)
            t640_s[:, hs] = _dot_nt(wqT_s[...], h1) * (SCALE * LOG2E)
        expand(t640_s, pad_s)
        qt_s[pl.ds(pl.multiple_of(b * G, G), G)] = pad_s[...].astype(bf16)
        return carry

    with jax.named_scope('phase_a'):
        jax.lax.fori_loop(0, NB, phase_a, 0)

    cp_wmod1.start()
    cp_wo.start()
    cp_w1.start()
    cp_w2.start()
    g_copy(0).start()

    grow_id = jax.lax.broadcasted_iota(jnp.int32, (DQ, GW), 0)
    row8 = jax.lax.broadcasted_iota(jnp.int32, (8, GW), 0)
    hrow = jax.lax.broadcasted_iota(jnp.int32, (H, D), 0)
    hcol = jax.lax.broadcasted_iota(jnp.int32, (H, D), 1)
    head_ind = jnp.where((hcol >= hrow * DH) & (hcol < (hrow + 1) * DH),
                         1.0, 0.0).astype(bf16)

    def finish_o(gc, o):
        inv_l = 1.0 / o[DH:DH + 1, :]
        invl_s[gc] = inv_l
        ot_s[gc] = jnp.where(grow_id < DH, o * inv_l, 0.0)

    def fwd_groups(b, tc, us, produce):
        pend = None
        o = None

        def flush(pend, o):
            gc, sl, p, is_last = pend
            oo = _dot_nn(vT_s[:, sl], p)
            o = oo if o is None else o + oo
            if is_last:
                finish_o(gc, o)
                o = None
            return o

        for u in us:
            if produce:
                qn = qt_s[b * G + (tc + 1) * FU + u]
            gc = tc * FU + u
            mc = m_s[u]
            m8 = None
            for ck in range(NC):
                sl = slice(ck * CK, (ck + 1) * CK)
                p = jnp.exp2(s_s[u, sl, :] - mc).astype(bf16)
                p_s[gc, sl, :] = p
                if produce:
                    s = _dot(kaug_s[sl, :], qn)
                    s_s[u, sl, :] = s
                    mm = jnp.max(s.reshape(CK // 8, 8, GW), axis=0)
                    m8 = mm if m8 is None else jnp.maximum(m8, mm)
                if pend is not None:
                    o = flush(pend, o)
                pend = (gc, sl, p, ck == NC - 1)
            if produce:
                m_s[u] = jnp.max(m8, axis=0, keepdims=True)
        flush(pend, o)

    def bwd_group(b, gg):
        dp = dp_s[...]
        for u in range(BU):
            g = gg * BU + u
            q = qt_s[b * G + g].astype(f32)[0:DQ]
            do = dot_s[g]
            do32 = do.astype(f32)[0:DQ]
            dq = None
            for ck in range(NC):
                sl = slice(ck * CK, (ck + 1) * CK)
                p = p_s[g, sl, :]
                ds = (p.astype(f32) * dp).astype(bf16)
                if ck + 1 < NC:
                    dp = _dot(vaug_s[(ck + 1) * CK:(ck + 2) * CK, :], do)
                else:
                    gnext = jnp.minimum(g + 1, G - 1)
                    dp = _dot(vaug_s[0:CK, :], dot_s[gnext])
                dv = None
                for j in range(NJ):
                    js = slice(j * 128, (j + 1) * 128)
                    t = _dot_nt(do32[:, js], p[:, js])
                    dv = t if dv is None else dv + t
                dk = None
                for j in range(NJ):
                    js = slice(j * 128, (j + 1) * 128)
                    t = _dot_nt(q[:, js], ds[:, js])
                    dk = t if dk is None else dk + t
                dvT_s[:, sl] += dv
                dkT_s[:, sl] += dk
                d = _dot_nn(kT_s[:, sl], ds)
                dq = d if dq is None else dq + d
            dqt_s[g] = dq
        dp_s[...] = dp

    def fchunk(j):
        if isinstance(j, int):
            return slice(j * FC, (j + 1) * FC)
        return pl.ds(pl.multiple_of(j * FC, FC), FC)

    def ffn_act(u, da):
        sig = _sigmoid(u)
        a = (u * sig).astype(bf16)
        du = (da * (sig * (1.0 + u * (1.0 - sig)))).astype(bf16)
        return a, du

    def dq_compact():
        compact(dqt_s, t640b_s)
        return (t640b_s[...] * SCALE).astype(bf16)

    def phase_b(b, carry):
        rows = blk(b)
        prev = blk(jnp.maximum(b - 1, 0))

        def fwd_body(t, cc):
            fwd_groups(b, t, range(FU), True)
            return cc

        with jax.named_scope('fwd_loop'):
            jax.lax.fori_loop(0, jnp.where(b == NB - 1, G // FU - 1, G // FU), fwd_body, 0)

        @pl.when(b == NB - 1)
        def _():
            def fwd_epi(u, cc):
                fwd_groups(b, G // FU - 1, [u], False)
                return cc

            jax.lax.fori_loop(0, FU, fwd_epi, 0)

        @pl.when(b == 0)
        def _():
            cp_wmod1.wait()
            mod_s[:, 2 * D:6 * D] = _dot(silu_b, wmod_ref[:, 2 * D:6 * D])
            cp_wo.wait()
            cp_w1.wait()
            cp_w2.wait()

        g_copy(b).wait()

        @pl.when(b + 1 < NB)
        def _():
            g_copy(b + 1).start()

        gb_ref = g_ref.at[b % 2]

        compact(ot_s, t640_s)
        ob = t640_s[...].T.astype(bf16)
        dqT = dq_compact()
        dq = dqT.T

        ga, sb, cb, gb = mod(2), mod(3), mod(4), mod(5)
        df = (gb_ref[...].astype(f32) * gb).astype(bf16)
        df_s[...] = df
        da = _dot_nt(df, w2_ref[fchunk(0), :])

        def act0(rc0):
            r2 = slice(rc0 * RC, (rc0 + 2) * RC)
            u = _dot_nt(h2_s[r2, :], w1T_ref[fchunk(0), :])
            a, du = ffn_act(u, da[r2, :])
            a_s[r2, :] = a
            du_s[r2, :] = du

        for rc in range(NRC):
            rs = slice(rc * RC, (rc + 1) * RC)
            attn = _dot(ob[rs, :], wo_ref[...])
            at_s[rs, :] = attn
            x1 = x_ref[rchunk(b, rc), :].astype(f32) + ga * attn
            xhat2, rstd2 = _ln_stats(x1)
            h2_s[rs, :] = (xhat2 * (1.0 + cb) + sb).astype(bf16)
            x1_s[rs, :] = x1
            xh_s[rs, :] = xhat2
            rstd_s[rs, :] = rstd2
            if rc < ND:
                ns = slice(rc * 128, (rc + 1) * 128)
                dh1_s[prev, ns] = _dot(dq, wqT_s[:, ns])
            else:
                ms = slice((rc - ND) * 128, (rc - ND + 1) * 128)
                dwqT_s[ms, :] += _dot(dqT[ms, :], h1_s[prev, :])
            if rc % 2 == 1 and rc >= 3:
                act0(rc - 3)
        ms = slice((NRC - ND) * 128, (NRC - ND + 1) * 128)
        dwqT_s[ms, :] += _dot(dqT[ms, :], h1_s[prev, :])
        act0(NRC - 2)
        ms = slice((NRC - ND + 1) * 128, D)
        dwqT_s[ms, :] += _dot(dqT[ms, :], h1_s[prev, :])

        def ffn(jj, cc):
            h2v = h2_s[...]
            dfv = df_s[...]
            a = a_s[...]
            du = du_s[...]
            for k in range(FUN):
                j = jj * FUN + k
                fs = fchunk(j)
                fn = fchunk(j + 1)
                if k == 0:
                    f_s[...] = jnp.where(j > 0, f_s[...], 0.0) + _dot(a, w2_ref[fs, :])
                    dh2_s[...] = jnp.where(j > 0, dh2_s[...], 0.0) + _dot(du, w1T_ref[fs, :])
                else:
                    f_s[...] += _dot(a, w2_ref[fs, :])
                    dh2_s[...] += _dot(du, w1T_ref[fs, :])
                un = _dot_nt(h2v, w1T_ref[fn, :])
                dan = _dot_nt(dfv, w2_ref[fn, :])
                an, dun = ffn_act(un, dan)
                if k == FUN - 1:
                    a_s[...] = an
                    du_s[...] = dun
                t = dw2_s[fs, :] + _dot_tn(a, dfv)
                dw2_s[fs, :] = t
                dw2_ref[fs, :] = t.astype(bf16)
                t = dw1_s[fs, :] + _dot_tn(du, h2v)
                dw1_s[fs, :] = t
                dw1T_ref[fs, :] = t.astype(bf16)
                a, du = an, dun
            return cc

        with jax.named_scope('ffn'):
            jax.lax.fori_loop(0, (NF - 1) // FUN, ffn, 0)

        fs = fchunk(NF - 1)
        a = a_s[...]
        du = du_s[...]
        FL = F - (NF - 1) * FC
        fl = slice((NF - 1) * FC, F)
        aT = a.T[0:FL, :]
        duT = du.T[0:FL, :]

        R3 = 64
        npc = 0
        for rc in range(TQ // R3):
            rs = slice(rc * R3, (rc + 1) * R3)
            rr = pl.ds(pl.multiple_of(b * TQ + rc * R3, R3), R3)
            dh2 = dh2_s[rs, :] + _dot(du[rs, :], w1T_ref[fs, :])
            f = f_s[rs, :] + _dot(a[rs, :], w2_ref[fs, :])
            xhat2 = xh_s[rs, :]
            gr = gb_ref[rs, :].astype(f32)
            out_ref[rr, :] = (x1_s[rs, :] + gb * f).astype(out_ref.dtype)
            dmod_s[:, 5 * D:6 * D] += _colsum8(gr * f)
            dmod_s[:, 3 * D:4 * D] += _colsum8(dh2)
            dmod_s[:, 4 * D:5 * D] += _colsum8(dh2 * xhat2)
            dx1 = gr + _ln_bwd(dh2 * (1.0 + cb), xhat2, rstd_s[rs, :])
            dx1_s[rr, :] = dx1
            dmod_s[:, 2 * D:3 * D] += _colsum8(dx1 * at_s[rs, :])
            dat_s[rs, :] = (dx1 * ga).astype(bf16)
            for _k in range(2 if rc == TQ // R3 - 1 else 1):
                ns = slice(npc * 128, (npc + 1) * 128)
                npc += 1
                t = dw2_s[fl, ns] + _dot(aT, df_s[:, ns])
                dw2_s[fl, ns] = t
                dw2_ref[fl, ns] = t.astype(bf16)
                t = dw1_s[fl, ns] + _dot(duT, h2_s[:, ns])
                dw1_s[fl, ns] = t
                dw1T_ref[fl, ns] = t.astype(bf16)
        out_copy(b).start()
        dattn = dat_s[...]
        t640b_s[...] = _dot_nt(wo_ref[...], dattn)
        t = dwo_s[0:256, :] + _dot(t640_s[0:256, :].astype(bf16), dattn)
        dwo_s[0:256, :] = t
        dwo_ref[0:256, :] = t.astype(bf16)
        expand(t640b_s, pad_s)
        prod = t640b_s[...] * t640_s[...]
        prod_hi = prod.astype(bf16)
        prod_lo = (prod - prod_hi.astype(f32)).astype(bf16)
        delta = _dot(head_ind, prod_hi) + _dot(head_ind, prod_lo)
        for hh in range(H):
            g, j = hh // HG, hh % HG
            pad_s[g, DH:DH + 1, j * TQ:(j + 1) * TQ] = -delta[hh:hh + 1, :]

        for g in range(G):
            v = pad_s[g] * invl_s[g]
            top = v[16:24, :]
            r1 = top - top.astype(bf16).astype(f32)
            r2 = r1 - r1.astype(bf16).astype(f32)
            top = jnp.where(row8 == DH + 1 - 16, pltpu.roll(r1, 1, 0),
                            jnp.where(row8 == DH + 2 - 16, pltpu.roll(r2, 2, 0), top))
            dot_s[g] = jnp.concatenate([v[0:16], top, v[24:32]], axis=0).astype(bf16)

        t = dwo_s[256:D, :] + _dot(t640_s[256:D, :].astype(bf16), dattn)
        dwo_s[256:D, :] = t
        dwo_ref[256:D, :] = t.astype(bf16)
        dp_s[...] = _dot(vaug_s[0:CK, :], dot_s[0])

        @pl.when(b == NB - 1)
        def _():
            cp_dwo.start()
            cp_dw1.start()
            cp_dw2.start()
            dmr = _colsum(dmod_s[:, 2 * D:6 * D])
            dsl_s[...] = _dot_nt(dmr.astype(bf16), wmod_ref[:, 2 * D:6 * D])
            sc = scol_s[...]
            for n in range(4 * ND):
                ns = slice((2 * ND + n) * 128, (2 * ND + n + 1) * 128)
                wmod_ref[:, ns] = (sc * dmr[:, n * 128:(n + 1) * 128]).astype(bf16)
            cp_dwmod1.start()

        def bwd_body(gg, cc):
            bwd_group(b, gg)
            return cc

        with jax.named_scope('bwd_loop'):
            jax.lax.fori_loop(0, NBL, bwd_body, 0)
        return carry

    def fwd_pro(u, cc):
        qn = qt_s[u]
        m8 = None
        for ck in range(NC):
            sl = slice(ck * CK, (ck + 1) * CK)
            sv = _dot(kaug_s[sl, :], qn)
            s_s[u, sl, :] = sv
            mm = jnp.max(sv.reshape(CK // 8, 8, GW), axis=0)
            m8 = mm if m8 is None else jnp.maximum(m8, mm)
        m_s[u] = jnp.max(m8, axis=0, keepdims=True)
        return cc

    jax.lax.fori_loop(0, FU, fwd_pro, 0)
    with jax.named_scope('phase_b'):
        jax.lax.fori_loop(0, NB, phase_b, 0)

    last = slice((NB - 1) * TQ, NB * TQ)
    dqT = dq_compact()
    dh1_s[last, :] = _dot_tn(dqT, wqT_s[...])
    dwqT_s[...] += _dot(dqT, h1_s[last, :])

    dwq_ref[...] = dwqT_s[...].T.astype(dwq_ref.dtype)
    cp_dwq.start()
    srow_id = jax.lax.broadcasted_iota(jnp.int32, (DQ, S), 0)
    dkT = _r32(jnp.where(srow_id < DH, dkT_s[...] * LN2, 0.0))
    dvT = _r32(jnp.where(srow_id < DH, dvT_s[...], 0.0))
    z8 = jnp.zeros((DP - DQ, S), f32)
    kaug_s[...] = jnp.concatenate([dkT, z8], axis=0).T.astype(bf16)
    vaug_s[...] = jnp.concatenate([dvT, z8], axis=0).T.astype(bf16)
    dwkT = _dot_nn(dkT, h1_s[...])
    dwvT = _dot_nn(dvT, h1_s[...])
    dwkT_ref[...] = dwkT[0:DH, :].astype(dwkT_ref.dtype)
    dwvT_ref[...] = dwvT[0:DH, :].astype(dwvT_ref.dtype)

    def phase_c(b, carry):
        out_copy(b).wait()
        ca1 = 1.0 + mod(1)
        for hf in range(TQ // 64):
            hr = pl.ds(pl.multiple_of(b * TQ + hf * 64, 64), 64)
            dh1 = dh1_s[hr, :] + _dot(kaug_s[hr, :], wkvT_s[0:DP, :]) \
                + _dot(vaug_s[hr, :], wkvT_s[DP:2 * DP, :])
            xhat = xh1_s[hr, :]
            dmod_s[:, 0:D] += _colsum8(dh1)
            dmod_s[:, D:2 * D] += _colsum8(dh1 * xhat)
            dx = dx1_s[hr, :] + _ln_bwd(dh1 * ca1, xhat, rstd1_s[hr, :])
            dx_ref[hr, :] = dx.astype(dx_ref.dtype)
        dx_copy(b).start()
        return carry + 1

    with jax.named_scope('phase_c'):
        nblk = jax.lax.fori_loop(0, NB, phase_c, 0)

    dmod32 = _colsum(dmod_s[:, 0:2 * D])
    sc = scol_s[...]
    for n in range(2 * ND):
        ns = slice(n * 128, (n + 1) * 128)
        dwmod_ref[:, ns] = (sc * dmod32[:, ns]).astype(bf16)
    cp_dwmod0.start()

    @pl.when(nblk > 0)
    def _():
        dmod0 = _colsum(dmod_s[:, 0:2 * D]).astype(bf16)
        dsilu = dsl_s[...] + _dot_nt(dmod0, wmod_ref[:, 0:2 * D])
        dc_ref[...] = (dsilu * (sig_c * (1.0 + c * (1.0 - sig_c)))).astype(dc_ref.dtype)

    for b in range(NB):
        dx_copy(b).wait()
    cp_dwq.wait()
    cp_dwo.wait()
    cp_dw1.wait()
    cp_dw2.wait()
    cp_dwmod0.wait()
    cp_dwmod1.wait()


@jax.jit
def pallas_adaLN_cond__grouped_kv_mqa__dense_activation_silu__prompt_kernel(
    A_x: jax.Array,
    A_wq: jax.Array,
    A_wk: jax.Array,
    A_wv: jax.Array,
    A_wo: jax.Array,
    B_x: jax.Array,
    B_w1: jax.Array,
    B_w2: jax.Array,
    c: jax.Array,
    w_mod: jax.Array,
    grad_out: jax.Array,
):
    x = A_x.reshape(S, D)
    g = grad_out.reshape(S, D)
    sds = jax.ShapeDtypeStruct
    out_shape = (
        sds((S, D), bf16),
        sds((S, D), bf16),
        sds((D, D), bf16),
        sds((DH, D), bf16),
        sds((DH, D), bf16),
        sds((D, D), bf16),
        sds((F, D), bf16),
        sds((F, D), bf16),
        sds((1, D), bf16),
        sds((D, 6 * D), bf16),
    )
    V = pltpu.VMEM
    DMA = pltpu.SemaphoreType.DMA
    scratch = [
        V((S, D), bf16),
        V((D, D), bf16),
        V((FP, D), bf16),
        V((FP, D), bf16),
        V((D, 6 * D), bf16),
        V((2, TQ, D), bf16),
        V((S, D), bf16),
        V((D, D), bf16),
        V((D, D), bf16),
        V((F, D), bf16),
        V((F, D), bf16),
        V((D, 2 * D), bf16),
        DMA((6,)),
        DMA((2,)),
        DMA((NB,)),
        DMA((NB,)),
        DMA((NB,)),
        DMA((6,)),
        V((1, 6 * D), f32),
        V((S, D), bf16),
        V((D, D), bf16),
        V((2 * DP, D), bf16),
        V((S, DP), bf16),
        V((S, DP), bf16),
        V((DQ, S), f32),
        V((DQ, S), f32),
        V((G, S, GW), bf16),
        V((FU, S, GW), f32),
        V((FU, 1, GW), f32),
        V((NB * G, DP, GW), bf16),
        V((G, DP, GW), f32),
        V((D, TQ), f32),
        V((G, DQ, GW), f32),
        V((G, 1, GW), f32),
        V((G, DP, GW), bf16),
        V((G, DQ, GW), f32),
        V((DQ, S), f32),
        V((DQ, S), f32),
        V((FP, D), f32),
        V((FP, D), f32),
        V((D, D), f32),
        V((D, D), f32),
        V((8, 6 * D), f32),
        V((S, D), f32),
        V((S, D), f32),
        V((CK, GW), f32),
        V((TQ, D), bf16),
        V((TQ, D), bf16),
        V((TQ, D), f32),
        V((TQ, D), f32),
        V((TQ, D), f32),
        V((TQ, D), f32),
        V((TQ, FC), bf16),
        V((TQ, FC), bf16),
        V((D, TQ), f32),
        V((TQ, D), f32),
        V((TQ, 1), f32),
        V((TQ, D), bf16),
        V((D, 128), f32),
        V((S, D), f32),
        V((S, 1), f32),
        V((1, D), f32),
    ]
    hbm = pl.BlockSpec(memory_space=pl.ANY)
    vm = pl.BlockSpec(memory_space=pltpu.VMEM)
    outs = pl.pallas_call(
        _kernel,
        out_shape=out_shape,
        in_specs=[hbm, hbm, vm, vm, hbm, hbm, hbm, vm, hbm, hbm],
        out_specs=(hbm, hbm, hbm, vm, vm, hbm, hbm, hbm, vm, hbm),
        scratch_shapes=scratch,
        compiler_params=pltpu.CompilerParams(
            vmem_limit_bytes=126 * 1024 * 1024),
    )(x, A_wq, A_wk.T, A_wv.T, A_wo, B_w1.T, B_w2, c, w_mod, g)
    out, dx = outs[0].reshape(1, S, D), outs[1].reshape(1, S, D)
    return (out, dx, outs[2], outs[3].T, outs[4].T, outs[5], outs[6].T,
            outs[7], outs[8], outs[9])
```
